```python
import os as _os
_os.environ.setdefault("JAX_PLATFORMS", "cpu")
import jax
import jax.numpy as jnp

def _softmax(x, axis=-1):
    return jax.nn.softmax(x, axis=axis)
def _gelu(x):
    return jax.nn.gelu(x, approximate=True)
def _silu(x):
    return jax.nn.silu(x)
def _sigmoid(x):
    return jax.nn.sigmoid(x)
def _layernorm(x, axis=-1, eps=1e-5):
    m = jnp.mean(x, axis=axis, keepdims=True)
    v = jnp.var(x, axis=axis, keepdims=True)
    return (x - m) / jnp.sqrt(v + eps)
def _scatter_add(tgt, idx, src, axis=0):
    return tgt.at[idx].add(src)
def _segment_sum(src, seg, n):
    return jax.ops.segment_sum(src, seg, n)
class _Rng:
    def __init__(self, key):
        self._k = key
    def _next(self):
        self._k, sub = jax.random.split(self._k)
        return sub
    def normal(self, shape):
        return jax.random.normal(self._next(), shape, dtype=jnp.bfloat16)
    def randint(self, lo, hi, shape):
        return jax.random.randint(self._next(), shape, lo, hi, dtype=jnp.int32)
    def uniform(self, shape, lo=0.0, hi=1.0):
        return jax.random.uniform(self._next(), shape, jnp.bfloat16, lo, hi)
    def permutation(self, n):
        return jax.random.permutation(self._next(), n)


kernel_name = 'gated_mix__ssm_conv_s5__geglu_ffn__prompt'

def setup_inputs():
    _rng = _Rng(jax.random.key(int.from_bytes(__import__("os").urandom(4), "little")))
    _w = (lambda a: (lambda t: t.astype(jnp.bfloat16) if jnp.issubdtype(t.dtype, jnp.floating) else t)(jnp.asarray(a)))
    def _A_setup():
        B, S, D = 1, 2048, 512
        P = D
        Lambda_re = -0.5 * jnp.exp((lambda *s: _rng.normal(s) * 0.4)(P))
        Lambda_im = (lambda *s: _rng.normal(s) * 0.4)(P) * 1.0
        B_re = (lambda *s: _rng.normal(s) * 0.4)(P, D) * (D ** -0.5)
        B_im = (lambda *s: _rng.normal(s) * 0.4)(P, D) * (D ** -0.5)
        C_re = (lambda *s: _rng.normal(s) * 0.4)(D, P) * (P ** -0.5)
        C_im = (lambda *s: _rng.normal(s) * 0.4)(D, P) * (P ** -0.5)
        log_dt = (lambda *s: _rng.normal(s) * 0.4)(P) * 0.3 - 2.0
        Dskip = (lambda *s: _rng.normal(s) * 0.4)(D)
        return {
            "x": _w((lambda *s: _rng.normal(s) * 0.05)(B, S, D)),
            "Lambda_re": _w(Lambda_re),
            "Lambda_im": _w(Lambda_im),
            "B_re": _w(B_re),
            "B_im": _w(B_im),
            "C_re": _w(C_re),
            "C_im": _w(C_im),
            "log_dt": _w(log_dt),
            "Dskip": _w(Dskip),
        }
    _A_in = _A_setup()

    def _B_setup():
        B, S, D, F = 1, 2048, 512, 1376
        return {
            "x": _w((lambda *s: _rng.normal(s) * 0.05)(B, S, D)),
            "w_gate": _w((lambda *s: _rng.normal(s) * 0.1)(D, F)),
            "w_up": _w((lambda *s: _rng.normal(s) * 0.1)(D, F)),
            "w_down": _w((lambda *s: _rng.normal(s) * 0.1)(F, D)),
        }
    _B_in = _B_setup()

    return {
        "A_x": _A_in["x"],
        "A_Lambda_re": _A_in["Lambda_re"],
        "A_Lambda_im": _A_in["Lambda_im"],
        "A_B_re": _A_in["B_re"],
        "A_B_im": _A_in["B_im"],
        "A_C_re": _A_in["C_re"],
        "A_C_im": _A_in["C_im"],
        "A_log_dt": _A_in["log_dt"],
        "A_Dskip": _A_in["Dskip"],
        "B_x": _B_in["x"],
        "B_w_gate": _B_in["w_gate"],
        "B_w_up": _B_in["w_up"],
        "B_w_down": _B_in["w_down"],
        "gate_w": _w((lambda *s: _rng.normal(s) * 0.05)(512) * 16.0),
    }

def reference(A_x, A_Lambda_re, A_Lambda_im, A_B_re, A_B_im, A_C_re, A_C_im, A_log_dt, A_Dskip, B_x, B_w_gate, B_w_up, B_w_down, gate_w):
    def _A_ref(x, Lambda_re, Lambda_im, B_re, B_im, C_re, C_im, log_dt, Dskip):
        Bsz, L, H = x.shape
        Lam = Lambda_re + 1j * Lambda_im
        Bmat = B_re + 1j * B_im
        Cmat = C_re + 1j * C_im
        dt = jnp.exp(log_dt)
        Lam_bar = jnp.exp(dt * Lam)
        B_bar = ((Lam_bar - 1.0) / Lam)[:, None] * Bmat
        Bu = jnp.einsum("bld,pd->blp", x + 0j, B_bar)
        h = jnp.zeros_like(Bu[:, 0, :])
        hs = []
        for t in range(L):
            h = Lam_bar[None, :] * h + Bu[:, t, :]
            hs.append(h)
        hseq = jnp.stack(hs, 1)
        y = 2.0 * jnp.einsum("blp,dp->bld", hseq, Cmat).real + x * Dskip[None, None, :]
        return y

    def _B_ref(x, w_gate, w_up, w_down):
        return (_gelu(x @ w_gate) * (x @ w_up)) @ w_down

    x = A_x
    g = _sigmoid((x * gate_w).sum(-1, keepdims=True))
    a = _A_ref(x, A_Lambda_re, A_Lambda_im, A_B_re, A_B_im, A_C_re, A_C_im, A_log_dt, A_Dskip)
    b = _B_ref(x, B_w_gate, B_w_up, B_w_down)
    return g * a + (1 - g) * b
```

```python
import functools

import jax
import jax.numpy as jnp
import jax.experimental.pallas as pl
import jax.experimental.pallas.tpu as pltpu

TB = 512
NSEG = 8


def _gelu_tanh(x):
    c = 0.7978845608028654
    return 0.5 * x * (1.0 + jnp.tanh(c * (x + 0.044715 * (x * x * x))))


def _kernel(x_ref, lre_ref, lim_ref, bre_ref, bim_ref, cre_ref, cim_ref, ldt_ref,
            dsk_ref, wg_ref, wu_ref, wd_ref, gw_ref, o_ref,
            cc_ref, a_ref, carry_ref, bu_ref, *, P):
    i = pl.program_id(0)
    SL = TB // NSEG

    @pl.when(i == 0)
    def _init():
        lre = lre_ref[...].astype(jnp.float32)
        lim = lim_ref[...].astype(jnp.float32)
        dt = jnp.exp(ldt_ref[...].astype(jnp.float32))
        dt = dt.astype(jnp.bfloat16).astype(jnp.float32)
        er = jnp.exp(dt * lre)
        zi = dt * lim
        a_re = er * jnp.cos(zi)
        a_im = er * jnp.sin(zi)
        den = lre * lre + lim * lim
        nr = a_re - 1.0
        ni = a_im
        co_re = (nr * lre + ni * lim) / den
        co_im = (ni * lre - nr * lim) / den
        cre = cre_ref[...].astype(jnp.float32)
        cim = cim_ref[...].astype(jnp.float32)
        cc_ref[:, 0:P] = (2.0 * (cre * co_re - cim * co_im)).astype(jnp.bfloat16)
        cc_ref[:, P:2 * P] = (-2.0 * (cre * co_im + cim * co_re)).astype(jnp.bfloat16)
        p_re, p_im = a_re, a_im
        n = SL
        while n > 1:
            p_re, p_im = p_re * p_re - p_im * p_im, 2.0 * p_re * p_im
            n //= 2
        a_ref[0:1, :] = a_re
        a_ref[1:2, :] = a_im
        a_ref[2:3, :] = p_re
        a_ref[3:4, :] = p_im
        carry_ref[...] = jnp.zeros_like(carry_ref)

    x = x_ref[...]
    nt = (((1,), (1,)), ((), ()))
    NJ = P // 128
    bur = jax.lax.dot_general(x, bre_ref[...], nt, preferred_element_type=jnp.float32)
    bui = jax.lax.dot_general(x, bim_ref[...], nt, preferred_element_type=jnp.float32)
    for j in range(NJ):
        bu_ref[j] = bur[:, j * 128:(j + 1) * 128]
        bu_ref[NJ + j] = bui[:, j * 128:(j + 1) * 128]

    def ld(k):
        rows = pl.ds(k, NSEG, stride=SL)
        b_re = jnp.concatenate([bu_ref[j, rows, :] for j in range(NJ)], axis=1)
        b_im = jnp.concatenate([bu_ref[NJ + j, rows, :] for j in range(NJ)], axis=1)
        return b_re, b_im

    def st(k, v_re, v_im):
        rows = pl.ds(k, NSEG, stride=SL)
        for j in range(NJ):
            bu_ref[j, rows, :] = v_re[:, j * 128:(j + 1) * 128]
            bu_ref[NJ + j, rows, :] = v_im[:, j * 128:(j + 1) * 128]

    a_re = jnp.broadcast_to(a_ref[0:1, :], (NSEG, P))
    a_im = jnp.broadcast_to(a_ref[1:2, :], (NSEG, P))
    s_re = a_ref[2:3, :]
    s_im = a_ref[3:4, :]

    def p1(k, e):
        e_re, e_im = e
        b_re, b_im = ld(k)
        n_re = a_re * e_re - a_im * e_im + b_re
        n_im = a_re * e_im + a_im * e_re + b_im
        return n_re, n_im

    z = jnp.zeros((NSEG, P), jnp.float32)
    e_re, e_im = jax.lax.fori_loop(0, SL, p1, (z, z), unroll=8)

    c_re = carry_ref[0:1, :]
    c_im = carry_ref[1:2, :]
    rows_re, rows_im = [], []
    for s in range(NSEG):
        rows_re.append(c_re)
        rows_im.append(c_im)
        n_re = s_re * c_re - s_im * c_im + e_re[s:s + 1, :]
        n_im = s_re * c_im + s_im * c_re + e_im[s:s + 1, :]
        c_re, c_im = n_re, n_im
    carry_ref[0:1, :] = c_re
    carry_ref[1:2, :] = c_im
    h0_re = jnp.concatenate(rows_re, axis=0)
    h0_im = jnp.concatenate(rows_im, axis=0)

    def p2(k, h):
        h_re, h_im = h
        b_re, b_im = ld(k)
        n_re = a_re * h_re - a_im * h_im + b_re
        n_im = a_re * h_im + a_im * h_re + b_im
        st(k, n_re, n_im)
        return n_re, n_im

    jax.lax.fori_loop(0, SL, p2, (h0_re, h0_im), unroll=8)

    h = jnp.concatenate([bu_ref[j].astype(jnp.bfloat16) for j in range(2 * NJ)], axis=1)
    y = jax.lax.dot_general(h, cc_ref[...], nt, preferred_element_type=jnp.float32)
    xf = x.astype(jnp.float32)
    a = y + xf * dsk_ref[...].astype(jnp.float32)

    gt = jnp.dot(x, wg_ref[...], preferred_element_type=jnp.float32)
    up = jnp.dot(x, wu_ref[...], preferred_element_type=jnp.float32)
    hh = (_gelu_tanh(gt) * up).astype(jnp.bfloat16)
    b = jnp.dot(hh, wd_ref[...], preferred_element_type=jnp.float32)

    g = jax.nn.sigmoid(jnp.sum(xf * gw_ref[...].astype(jnp.float32), axis=-1, keepdims=True))
    o_ref[...] = g * a + (1.0 - g) * b


@jax.jit
def pallas_gated_mix__ssm_conv_s5__geglu_ffn__prompt_kernel(
    A_x: jax.Array,
    A_Lambda_re: jax.Array,
    A_Lambda_im: jax.Array,
    A_B_re: jax.Array,
    A_B_im: jax.Array,
    A_C_re: jax.Array,
    A_C_im: jax.Array,
    A_log_dt: jax.Array,
    A_Dskip: jax.Array,
    B_x: jax.Array,
    B_w_gate: jax.Array,
    B_w_up: jax.Array,
    B_w_down: jax.Array,
    gate_w: jax.Array,
):
    Bsz, L, D = A_x.shape
    P = A_Lambda_re.shape[0]
    F = B_w_gate.shape[1]
    assert Bsz == 1 and L % TB == 0
    x = A_x.reshape(L, D)
    row = lambda v: v.reshape(1, -1)

    full = lambda shape: pl.BlockSpec(shape, lambda i: (0, 0))
    in_specs = [
        pl.BlockSpec((TB, D), lambda i: (i, 0)),
        full((1, P)), full((1, P)),
        full((P, D)), full((P, D)),
        full((D, P)), full((D, P)),
        full((1, P)), full((1, D)),
        full((D, F)), full((D, F)), full((F, D)),
        full((1, D)),
    ]
    out = pl.pallas_call(
        functools.partial(_kernel, P=P),
        grid=(L // TB,),
        in_specs=in_specs,
        out_specs=pl.BlockSpec((TB, D), lambda i: (i, 0)),
        out_shape=jax.ShapeDtypeStruct((L, D), jnp.float32),
        scratch_shapes=[
            pltpu.VMEM((D, 2 * P), jnp.bfloat16),
            pltpu.VMEM((8, P), jnp.float32),
            pltpu.VMEM((8, P), jnp.float32),
            pltpu.VMEM((2 * P // 128, TB, 128), jnp.float32),
        ],
        compiler_params=pltpu.CompilerParams(
            dimension_semantics=("arbitrary",),
            vmem_limit_bytes=100 * 1024 * 1024,
        ),
    )(x, row(A_Lambda_re), row(A_Lambda_im), A_B_re, A_B_im, A_C_re, A_C_im,
      row(A_log_dt), row(A_Dskip), B_w_gate, B_w_up, B_w_down, row(gate_w))
    return out.reshape(Bsz, L, D)
```

```python
import functools

import jax
import jax.numpy as jnp
import jax.experimental.pallas as pl
import jax.experimental.pallas.tpu as pltpu

TB = 512


def _gelu_tanh(x):
    c = 0.7978845608028654
    return 0.5 * x * (1.0 + jnp.tanh(c * (x + 0.044715 * (x * x * x))))


def _cmul(a_re, a_im, b_re, b_im):
    return a_re * b_re - a_im * b_im, a_re * b_im + a_im * b_re


def _kernel(x_ref, lre_ref, lim_ref, bre_ref, bim_ref, cre_hbm, cim_hbm, ldt_ref,
            dsk_ref, wg_hbm, wu_hbm, wd_hbm, gw_ref, o_ref,
            cre_ref, cim_ref, wg_ref, wu_ref, wd_ref, sem,
            cc_ref, a_ref, carry_ref, bu_ref, h_ref, *, P):
    i = pl.program_id(0)
    nt = (((1,), (1,)), ((), ()))

    srcs = (wg_hbm, wu_hbm, wd_hbm, cre_hbm, cim_hbm)
    dsts = (wg_ref, wu_ref, wd_ref, cre_ref, cim_ref)
    cps = [pltpu.make_async_copy(s, d, sem.at[k]) for k, (s, d) in enumerate(zip(srcs, dsts))]

    def disc():
        lre = lre_ref[...].reshape(1, P).astype(jnp.float32)
        lim = lim_ref[...].reshape(1, P).astype(jnp.float32)
        dt = jnp.exp(ldt_ref[...].reshape(1, P).astype(jnp.float32))
        dt = dt.astype(jnp.bfloat16).astype(jnp.float32)
        er = jnp.exp(dt * lre)
        zi = dt * lim
        a_re = er * jnp.cos(zi)
        a_im = er * jnp.sin(zi)
        return lre, lim, a_re, a_im

    def init_a():
        _, _, a_re, a_im = disc()
        pw = [(a_re, a_im)]
        for _ in range(7):
            pw.append(_cmul(pw[-1][0], pw[-1][1], a_re, a_im))
        sub = jax.lax.broadcasted_iota(jnp.int32, (8, P), 0)
        for lvl, sh in enumerate((1, 2, 4)):
            for c in range(2):
                a_ref[2 * lvl + c] = jnp.where(sub >= sh, jnp.broadcast_to(pw[sh - 1][c], (8, P)), 0.0)
        for c in range(2):
            a_ref[6 + c] = jnp.concatenate([pw[k][c] for k in range(8)], axis=0)
            a_ref[8 + c] = jnp.broadcast_to(pw[7][c], (8, P))
        carry_ref[...] = jnp.zeros_like(carry_ref)

    def init_c():
        lre, lim, a_re, a_im = disc()
        den = lre * lre + lim * lim
        nr = a_re - 1.0
        ni = a_im
        co_re = (nr * lre + ni * lim) / den
        co_im = (ni * lre - nr * lim) / den
        cre = cre_ref[...].astype(jnp.float32)
        cim = cim_ref[...].astype(jnp.float32)
        cc_ref[:, 0:P] = (2.0 * (cre * co_re - cim * co_im)).astype(jnp.bfloat16)
        cc_ref[:, P:2 * P] = (-2.0 * (cre * co_im + cim * co_re)).astype(jnp.bfloat16)

    def body(first):
        if first:
            for cp in cps:
                cp.start()
            init_a()

        x = x_ref[...]
        bu_ref[:, 0:P] = jax.lax.dot_general(x, bre_ref[...], nt, preferred_element_type=jnp.float32)
        bu_ref[:, P:2 * P] = jax.lax.dot_general(x, bim_ref[...], nt, preferred_element_type=jnp.float32)

        def scan():
            for j in range(P // 128):
                ls = slice(128 * j, 128 * j + 128)
                li = slice(P + 128 * j, P + 128 * j + 128)
                lv = [(a_ref[2 * l, :, ls], a_ref[2 * l + 1, :, ls]) for l in range(3)]
                ap_re, ap_im = a_ref[6, :, ls], a_ref[7, :, ls]
                c_re, c_im = carry_ref[0, :, ls], carry_ref[1, :, ls]
                for gg in range(TB // 16):
                    hr, hi = [], []
                    for g in (2 * gg, 2 * gg + 1):
                        v_re = bu_ref[8 * g:8 * g + 8, ls]
                        v_im = bu_ref[8 * g:8 * g + 8, li]
                        for lvl, sh in enumerate((1, 2, 4)):
                            r_re = pltpu.roll(v_re, sh, 0)
                            r_im = pltpu.roll(v_im, sh, 0)
                            m_re, m_im = _cmul(lv[lvl][0], lv[lvl][1], r_re, r_im)
                            v_re = v_re + m_re
                            v_im = v_im + m_im
                        t_re, t_im = _cmul(ap_re, ap_im, c_re, c_im)
                        v_re = v_re + t_re
                        v_im = v_im + t_im
                        hr.append(v_re)
                        hi.append(v_im)
                        c_re = jnp.broadcast_to(v_re[7:8, :], (8, 128))
                        c_im = jnp.broadcast_to(v_im[7:8, :], (8, 128))
                    h_ref[16 * gg:16 * gg + 16, ls] = jnp.concatenate(hr, axis=0).astype(jnp.bfloat16)
                    h_ref[16 * gg:16 * gg + 16, li] = jnp.concatenate(hi, axis=0).astype(jnp.bfloat16)
                carry_ref[0, :, ls] = c_re
                carry_ref[1, :, ls] = c_im

        if first:
            scan()
            cps[0].wait()
        gt = jax.lax.dot_general(x, wg_ref[...], nt, preferred_element_type=jnp.float32)
        if first:
            for cp in cps[1:]:
                cp.wait()
            init_c()
        up = jax.lax.dot_general(x, wu_ref[...], nt, preferred_element_type=jnp.float32)
        if not first:
            scan()
        hh = (_gelu_tanh(gt) * up).astype(jnp.bfloat16)
        b = jnp.dot(hh, wd_ref[...], preferred_element_type=jnp.float32)

        y = jax.lax.dot_general(h_ref[...], cc_ref[...], nt, preferred_element_type=jnp.float32)
        xf = x.astype(jnp.float32)
        a = y + xf * dsk_ref[...].reshape(1, P).astype(jnp.float32)

        g = jax.nn.sigmoid(jnp.sum(xf * gw_ref[...].reshape(1, P).astype(jnp.float32), axis=-1, keepdims=True))
        o_ref[...] = g * a + (1.0 - g) * b

    @pl.when(i == 0)
    def _():
        body(True)

    @pl.when(i > 0)
    def _():
        body(False)


@jax.jit
def pallas_gated_mix__ssm_conv_s5__geglu_ffn__prompt_kernel(
    A_x: jax.Array,
    A_Lambda_re: jax.Array,
    A_Lambda_im: jax.Array,
    A_B_re: jax.Array,
    A_B_im: jax.Array,
    A_C_re: jax.Array,
    A_C_im: jax.Array,
    A_log_dt: jax.Array,
    A_Dskip: jax.Array,
    B_x: jax.Array,
    B_w_gate: jax.Array,
    B_w_up: jax.Array,
    B_w_down: jax.Array,
    gate_w: jax.Array,
):
    Bsz, L, D = A_x.shape
    P = A_Lambda_re.shape[0]
    F = B_w_gate.shape[1]
    assert Bsz == 1 and L % TB == 0
    x = A_x.reshape(L, D)
    row = lambda v: v

    full = lambda shape: pl.BlockSpec(shape, lambda i: (0, 0))
    hbm = pl.BlockSpec(memory_space=pl.ANY)
    vec = lambda n: pl.BlockSpec((n,), lambda i: (0,))
    in_specs = [
        pl.BlockSpec((TB, D), lambda i: (i, 0)),
        vec(P), vec(P),
        full((P, D)), full((P, D)), hbm, hbm,
        vec(P), vec(D),
        hbm, hbm, hbm,
        vec(D),
    ]
    bf = jnp.bfloat16
    out = pl.pallas_call(
        functools.partial(_kernel, P=P),
        grid=(L // TB,),
        in_specs=in_specs,
        out_specs=pl.BlockSpec((TB, D), lambda i: (i, 0)),
        out_shape=jax.ShapeDtypeStruct((L, D), jnp.float32),
        scratch_shapes=[
            pltpu.VMEM((D, P), bf), pltpu.VMEM((D, P), bf),
            pltpu.VMEM((F, D), bf), pltpu.VMEM((F, D), bf), pltpu.VMEM((F, D), bf),
            pltpu.SemaphoreType.DMA((5,)),
            pltpu.VMEM((D, 2 * P), bf),
            pltpu.VMEM((10, 8, P), jnp.float32),
            pltpu.VMEM((2, 8, P), jnp.float32),
            pltpu.VMEM((TB, 2 * P), jnp.float32),
            pltpu.VMEM((TB, 2 * P), bf),
        ],
        compiler_params=pltpu.CompilerParams(
            dimension_semantics=("arbitrary",),
            vmem_limit_bytes=100 * 1024 * 1024,
        ),
    )(x, row(A_Lambda_re), row(A_Lambda_im), A_B_re, A_B_im, A_C_re, A_C_im,
      row(A_log_dt), row(A_Dskip), B_w_gate.T, B_w_up.T, B_w_down, row(gate_w))
    return out.reshape(Bsz, L, D)
```
